```python
import os as _os
_os.environ.setdefault("JAX_PLATFORMS", "cpu")
import jax
import jax.numpy as jnp

def _softmax(x, axis=-1):
    return jax.nn.softmax(x, axis=axis)
def _gelu(x):
    return jax.nn.gelu(x, approximate=True)
def _silu(x):
    return jax.nn.silu(x)
def _sigmoid(x):
    return jax.nn.sigmoid(x)
def _layernorm(x, axis=-1, eps=1e-5):
    m = jnp.mean(x, axis=axis, keepdims=True)
    v = jnp.var(x, axis=axis, keepdims=True)
    return (x - m) / jnp.sqrt(v + eps)
def _scatter_add(tgt, idx, src, axis=0):
    return tgt.at[idx].add(src)
def _segment_sum(src, seg, n):
    return jax.ops.segment_sum(src, seg, n)
class _Rng:
    def __init__(self, key):
        self._k = key
    def _next(self):
        self._k, sub = jax.random.split(self._k)
        return sub
    def normal(self, shape):
        return jax.random.normal(self._next(), shape, dtype=jnp.bfloat16)
    def randint(self, lo, hi, shape):
        return jax.random.randint(self._next(), shape, lo, hi, dtype=jnp.int32)
    def uniform(self, shape, lo=0.0, hi=1.0):
        return jax.random.uniform(self._next(), shape, jnp.bfloat16, lo, hi)
    def permutation(self, n):
        return jax.random.permutation(self._next(), n)


kernel_name = 'parallel_sum__softmax_full_mha__moe_arch_mod__prompt'

def setup_inputs():
    _rng = _Rng(jax.random.key(int.from_bytes(__import__("os").urandom(4), "little")))
    _w = (lambda a: (lambda t: t.astype(jnp.bfloat16) if jnp.issubdtype(t.dtype, jnp.floating) else t)(jnp.asarray(a)))
    def _A_setup():
        B, S, D = 1, 2048, 512
        return {
            "x": _w((lambda *s: _rng.normal(s) * 0.05)(B, S, D)),
            "wqkv": _w((lambda *s: _rng.normal(s) * 0.1)(D, 3 * D)),
            "wo": _w((lambda *s: _rng.normal(s) * 0.05)(D, D)),
        }
    _A_in = _A_setup()

    def _B_setup():
        B, S, D, F, C = 1, 2048, 512, 1792, 1
        return {
            "x": _w((lambda *s: _rng.normal(s) * 0.05)(B, S, D)),
            "w_r": _w((lambda *s: _rng.normal(s) * 1.6)(D)),
            "w_gate": _w((lambda *s: _rng.normal(s) * 0.1)(D, F)),
            "w_up": _w((lambda *s: _rng.normal(s) * 0.1)(D, F)),
            "w_down": _w((lambda *s: _rng.normal(s) * 0.1)(F, D)),
        }
    _B_in = _B_setup()

    return {
        "A_x": _A_in["x"],
        "A_wqkv": _A_in["wqkv"],
        "A_wo": _A_in["wo"],
        "B_x": _B_in["x"],
        "B_w_r": _B_in["w_r"],
        "B_w_gate": _B_in["w_gate"],
        "B_w_up": _B_in["w_up"],
        "B_w_down": _B_in["w_down"],
    }

def reference(A_x, A_wqkv, A_wo, B_x, B_w_r, B_w_gate, B_w_up, B_w_down):
    def _A_ref(x, wqkv, wo):
        B, S, D = x.shape
        H = 32; Dh = D // H
        qkv = (lambda x, *d: x.transpose(*d))((x @ wqkv).reshape(B, S, 3, H, Dh), 2, 0, 3, 1, 4)
        q, k, v = qkv[0], qkv[1], qkv[2]
        scale = Dh ** -0.5
        scores = jnp.einsum("bhqd,bhkd->bhqk", q, k) * scale
        p = _softmax(scores, axis=-1)
        o = jnp.einsum("bhqk,bhkd->bhqd", p, v)
        return (lambda x, *d: x.transpose(*d))(o, 0, 2, 1, 3).reshape(B, S, D) @ wo

    def _B_ref(x, w_r, w_gate, w_up, w_down):
        B, S, D = x.shape
        C = 1
        r = x @ w_r
        idx = jnp.argsort(-r, axis=-1)[:, :C]
        idx_e = jnp.repeat(idx.reshape(B, C, 1), D, axis=2)
        x_sel = jnp.take_along_axis(x, idx_e, axis=1)
        g = _silu(x_sel @ w_gate)
        u = x_sel @ w_up
        y = (g * u) @ w_down
        r_sel = _sigmoid(jnp.take_along_axis(r, idx, axis=1))
        y = y * r_sel.reshape(B, C, 1)
        b_off = (jnp.arange(B) * S).reshape(B, 1)
        flat_idx = (idx + b_off).reshape(B * C)
        zero = (x * 0.0).reshape(B * S, D)
        upd = _scatter_add(zero, flat_idx, y.reshape(B * C, D), axis=0)
        return x + upd.reshape(B, S, D)

    x = A_x
    xn = _layernorm(x, axis=-1)
    return x + _A_ref(xn, A_wqkv, A_wo) + _B_ref(xn, B_w_r, B_w_gate, B_w_up, B_w_down)
```

```python
import math

import jax
import jax.numpy as jnp
import jax.experimental.pallas as pl
import jax.experimental.pallas.tpu as pltpu

_H = 32
_EPS = 1e-5
_BQ = 512
_CK = 128
_LAG = 2
_RC = 512
_L_LO = 2.0 ** -60
_L_HI = 2.0 ** 60
_BIG = 3.0e38

f32 = jnp.float32
bf16 = jnp.bfloat16


def _dot(a, b, ca, cb):
    return jax.lax.dot_general(a, b, (((ca,), (cb,)), ((), ())),
                               preferred_element_type=f32)


def _kernel(x_hbm, wqkv_hbm, wo_hbm, wr_ref, wg_hbm, wu_hbm, wd_hbm, out_hbm,
            x_v, xn_v, wqkv_v, wo_v, wg_v, wu_v, wd_v,
            k_v, qt_v, vt_v, r_v, ot_v, y_v, out_v, idx_s, sems, osems):
    S, D = x_v.shape
    Dh = D // _H
    HG = 128 // Dh
    NG = D // 128
    NC = S // _RC
    NB = S // _BQ
    qscale = (Dh ** -0.5) * math.log2(math.e)

    def x_copy(c):
        return pltpu.make_async_copy(x_hbm.at[0, pl.ds(c * _RC, _RC), :],
                                     x_v.at[pl.ds(c * _RC, _RC), :], sems.at[c])

    wqkv_copy = pltpu.make_async_copy(wqkv_hbm, wqkv_v, sems.at[NC])
    wo_copy = pltpu.make_async_copy(wo_hbm, wo_v, sems.at[NC + 1])
    wg_copy = pltpu.make_async_copy(wg_hbm, wg_v, sems.at[NC + 2])
    wu_copy = pltpu.make_async_copy(wu_hbm, wu_v, sems.at[NC + 3])
    wd_copy = pltpu.make_async_copy(wd_hbm, wd_v, sems.at[NC + 4])

    wqkv_copy.start()
    for c in range(NC):
        x_copy(c).start()

    wqkv_copy.wait()
    wqv_t = jnp.concatenate(
        [wqkv_v[:, 0:D].T, wqkv_v[:, 2 * D:3 * D].T,
         jnp.broadcast_to(wr_ref[...].reshape(1, D), (16, D))], axis=0)
    for c in range(NC):
        rows = pl.ds(c * _RC, _RC)
        x_copy(c).wait()
        if c == NC - 1:
            wo_copy.start()
            wg_copy.start()
            wu_copy.start()
            wd_copy.start()
        x = x_v[rows, :].astype(f32)
        m = jnp.mean(x, axis=1, keepdims=True)
        xc = x - m
        var = jnp.mean(xc * xc, axis=1, keepdims=True)
        xn = (xc * jax.lax.rsqrt(var + _EPS)).astype(bf16)
        xn_v[rows, :] = xn
        kk = _dot(xn, wqkv_v[:, D:2 * D], 1, 0).astype(bf16)
        for g in range(NG):
            k_v[g, rows, :] = kk[:, g * 128:(g + 1) * 128]
        t = _dot(wqv_t, xn, 1, 1)
        for g in range(NG):
            qt_v[g, :, rows] = (t[g * 128:(g + 1) * 128, :] * qscale).astype(bf16)
            vt_v[g, :, rows] = t[D + g * 128:D + (g + 1) * 128, :].astype(bf16)
        r_v[:, rows] = t[2 * D:2 * D + 8, :]

    r = r_v[...].astype(bf16).astype(f32)
    rmax = jnp.max(r)
    lane = jax.lax.broadcasted_iota(jnp.int32, r.shape, 1)
    idx = jnp.min(jnp.where(r == rmax, lane, S))
    idx = jnp.minimum(idx, S - 1)
    idx_s[0] = idx

    def ffn():
        idx = idx_s[0]
        base = pl.multiple_of((idx // 16) * 16, 16)
        tile = xn_v[pl.ds(base, 16), :].astype(f32)
        sub = jax.lax.broadcasted_iota(jnp.int32, tile.shape, 0)
        xs = jnp.sum(jnp.where(sub == idx - base, tile, 0.0), axis=0, keepdims=True)
        xs = jnp.broadcast_to(xs, (16, D)).astype(bf16)
        wg_copy.wait()
        gate = _dot(xs, wg_v[...], 1, 0)
        wu_copy.wait()
        up = _dot(xs, wu_v[...], 1, 0)
        hid = (gate * jax.nn.sigmoid(gate) * up).astype(bf16)
        wd_copy.wait()
        y = _dot(hid, wd_v[...], 1, 0)
        y_v[...] = y[0:8, :] * jax.nn.sigmoid(jnp.broadcast_to(rmax, (8, D)))

    nck = S // _CK
    steps = [(h, j) for h in range(HG) for j in range(nck)]

    def attn_fast(g, q0, bad):
        qts = {}

        def qk(h, j):
            if h not in qts:
                qts[h] = qt_v[g, h * Dh:(h + 1) * Dh, pl.ds(q0, _BQ)]
            kh = k_v[g, j * _CK:(j + 1) * _CK, h * Dh:(h + 1) * Dh]
            p = jnp.exp2(_dot(kh, qts[h], 1, 0))
            return p.reshape(_CK // 8, 8, _BQ).sum(axis=0), p.astype(bf16)

        pend = {t: qk(*steps[t]) for t in range(_LAG)}
        o = l = None
        for t, (h, j) in enumerate(steps):
            if t + _LAG < len(steps):
                pend[t + _LAG] = qk(*steps[t + _LAG])
            ps, pb = pend.pop(t)
            pv = _dot(vt_v[g, h * Dh:(h + 1) * Dh, j * _CK:(j + 1) * _CK], pb, 1, 0)
            o = pv if j == 0 else o + pv
            l = ps if j == 0 else l + ps
            if j == nck - 1:
                l = l.sum(axis=0, keepdims=True)
                on = o / l
                ot_v[g, h * Dh:(h + 1) * Dh, :] = on.astype(bf16)
                ok = (l >= _L_LO) & (l <= _L_HI)
                ok = ok & (jnp.abs(on[0:8]) <= _BIG) & (jnp.abs(on[8:16]) <= _BIG)
                bad = jnp.where(ok, bad, 1.0)
        return bad

    def attn_safe(hh, q0):
        g = hh // HG
        r0 = pl.multiple_of((hh % HG) * Dh, Dh)
        qt = qt_v[g, :, pl.ds(q0, _BQ)]
        row = jax.lax.broadcasted_iota(jnp.int32, qt.shape, 0)
        qm = jnp.where((row >= r0) & (row < r0 + Dh), qt, jnp.zeros_like(qt))
        s = _dot(k_v[g], qm, 1, 0)
        p = jnp.exp2(s - jnp.max(s, axis=0, keepdims=True))
        l = jnp.sum(p, axis=0, keepdims=True)
        o = _dot(vt_v[g, pl.ds(r0, Dh), :], p.astype(bf16), 1, 0)
        ot_v[g, pl.ds(r0, Dh), :] = (o / l).astype(bf16)

    def out_copy(b, slot):
        return pltpu.make_async_copy(
            out_v.at[slot], out_hbm.at[0, pl.ds(b * _BQ, _BQ), :], osems.at[slot])

    def block(b, carry):
        q0 = pl.multiple_of(b * _BQ, _BQ)
        bad = jax.lax.fori_loop(0, NG, lambda g, bd: attn_fast(g, q0, bd),
                                jnp.zeros((8, _BQ), f32))

        @pl.when(jnp.max(bad) > 0.0)
        def _():
            jax.lax.fori_loop(0, _H, lambda hh, c: (attn_safe(hh, q0), c)[1], 0)

        @pl.when(b == 0)
        def _():
            wo_copy.wait()
            ffn()

        slot = b % 2

        @pl.when(b >= 2)
        def _():
            out_copy(b - 2, slot).wait()

        a = _dot(ot_v[...].reshape(D, _BQ), wo_v[...], 0, 0)
        rows = pl.ds(q0, _BQ)
        res = x_v[rows, :].astype(f32) + a + xn_v[rows, :].astype(f32)
        rid = jax.lax.broadcasted_iota(jnp.int32, (_BQ, D), 0) + q0
        res = res + jnp.where(rid == idx_s[0], y_v[0:1, :], 0.0)
        out_v[slot] = res.astype(bf16)
        out_copy(b, slot).start()
        return carry

    jax.lax.fori_loop(0, NB, block, 0)
    for b in range(max(NB - 2, 0), NB):
        out_copy(b, b % 2).wait()


@jax.jit
def pallas_parallel_sum__softmax_full_mha__moe_arch_mod__prompt_kernel(
    A_x: jax.Array,
    A_wqkv: jax.Array,
    A_wo: jax.Array,
    B_x: jax.Array,
    B_w_r: jax.Array,
    B_w_gate: jax.Array,
    B_w_up: jax.Array,
    B_w_down: jax.Array,
):
    del B_x
    _, S, D = A_x.shape
    F = B_w_gate.shape[1]
    NG = D // 128
    hbm = pl.BlockSpec(memory_space=pl.ANY)
    vmem = pl.BlockSpec(memory_space=pltpu.VMEM)
    scratch = [
        pltpu.VMEM((S, D), bf16),
        pltpu.VMEM((S, D), bf16),
        pltpu.VMEM((D, 3 * D), bf16),
        pltpu.VMEM((D, D), bf16),
        pltpu.VMEM((D, F), bf16),
        pltpu.VMEM((D, F), bf16),
        pltpu.VMEM((F, D), bf16),
        pltpu.VMEM((NG, S, 128), bf16),
        pltpu.VMEM((NG, 128, S), bf16),
        pltpu.VMEM((NG, 128, S), bf16),
        pltpu.VMEM((8, S), f32),
        pltpu.VMEM((NG, 128, _BQ), bf16),
        pltpu.VMEM((8, D), f32),
        pltpu.VMEM((2, _BQ, D), bf16),
        pltpu.SMEM((1,), jnp.int32),
        pltpu.SemaphoreType.DMA((S // _RC + 5,)),
        pltpu.SemaphoreType.DMA((2,)),
    ]
    return pl.pallas_call(
        _kernel,
        out_shape=jax.ShapeDtypeStruct(A_x.shape, A_x.dtype),
        in_specs=[hbm, hbm, hbm, vmem, hbm, hbm, hbm],
        out_specs=hbm,
        scratch_shapes=scratch,
        compiler_params=pltpu.CompilerParams(vmem_limit_bytes=100 * 2 ** 20),
    )(A_x, A_wqkv, A_wo, B_w_r, B_w_gate, B_w_up, B_w_down)
```

```python
import math

import jax
import jax.numpy as jnp
import jax.experimental.pallas as pl
import jax.experimental.pallas.tpu as pltpu

_H = 32
_EPS = 1e-5
_BQ = 512
_CK = 128
_LAG = 2
_GU = 2
_RC = 512
_L_LO = 2.0 ** -60
_L_HI = 2.0 ** 60
_BIG = 3.0e38

f32 = jnp.float32
bf16 = jnp.bfloat16


def _dot(a, b, ca, cb):
    return jax.lax.dot_general(a, b, (((ca,), (cb,)), ((), ())),
                               preferred_element_type=f32)


def _kernel(x_hbm, wqkv_hbm, wo_hbm, wr_ref, wg_hbm, wu_hbm, wd_hbm, out_hbm,
            x_v, xn_v, wqkv_v, wo_v, wg_v, wu_v, wd_v,
            k_v, qt_v, vt_v, r_v, ot_v, pp_v, pl_v, y_v, out_v, idx_s, sems, osems):
    S, D = x_v.shape
    Dh = D // _H
    HG = 128 // Dh
    NG = D // 128
    NC = S // _RC
    NB = S // _BQ
    qscale = (Dh ** -0.5) * math.log2(math.e)

    def x_copy(c):
        return pltpu.make_async_copy(x_hbm.at[0, pl.ds(c * _RC, _RC), :],
                                     x_v.at[pl.ds(c * _RC, _RC), :], sems.at[c])

    def w_copy(i):
        return pltpu.make_async_copy(wqkv_hbm.at[:, pl.ds(i * D, D)],
                                     wqkv_v.at[i], sems.at[NC + 4 + i])

    wo_copy = pltpu.make_async_copy(wo_hbm, wo_v, sems.at[NC])
    wg_copy = pltpu.make_async_copy(wg_hbm, wg_v, sems.at[NC + 1])
    wu_copy = pltpu.make_async_copy(wu_hbm, wu_v, sems.at[NC + 2])
    wd_copy = pltpu.make_async_copy(wd_hbm, wd_v, sems.at[NC + 3])

    x_copy(0).start()
    for i in (1, 0, 2):
        w_copy(i).start()
    for c in range(1, NC):
        x_copy(c).start()

    def layernorm(c):
        rows = pl.ds(c * _RC, _RC)
        x = x_v[rows, :].astype(f32)
        m = jnp.mean(x, axis=1, keepdims=True)
        xc = x - m
        var = jnp.mean(xc * xc, axis=1, keepdims=True)
        xn = (xc * jax.lax.rsqrt(var + _EPS)).astype(bf16)
        xn_v[rows, :] = xn
        return xn

    def proj_k(c, xn):
        kk = _dot(xn, wqkv_v[1], 1, 0).astype(bf16)
        for g in range(NG):
            k_v[g, pl.ds(c * _RC, _RC), :] = kk[:, g * 128:(g + 1) * 128]

    def proj_qv(c, xn):
        cols = pl.ds(c * _RC, _RC)
        t = _dot(wqv_t, xn, 1, 1)
        for g in range(NG):
            qt_v[g, :, cols] = (t[g * 128:(g + 1) * 128, :] * qscale).astype(bf16)
            vt_v[g, :, cols] = t[D + g * 128:D + (g + 1) * 128, :].astype(bf16)
        r_v[:, cols] = t[2 * D:2 * D + 8, :]

    x_copy(0).wait()
    xn = layernorm(0)
    w_copy(1).wait()
    proj_k(0, xn)
    w_copy(0).wait()
    w_copy(2).wait()
    wqv_t = jnp.concatenate(
        [wqkv_v[0].T, wqkv_v[2].T,
         jnp.broadcast_to(wr_ref[...].reshape(1, D), (16, D))], axis=0)
    for c in range(NC):
        if c + 1 < NC:
            x_copy(c + 1).wait()
        if c == min(1, NC - 1):
            wo_copy.start()
            wg_copy.start()
            wu_copy.start()
            wd_copy.start()
        if c > 0:
            proj_k(c, xn)
        xn_next = layernorm(c + 1) if c + 1 < NC else None
        proj_qv(c, xn)
        xn = xn_next

    r = r_v[...].astype(bf16).astype(f32)
    rmax = jnp.max(r)
    lane = jax.lax.broadcasted_iota(jnp.int32, r.shape, 1)
    idx = jnp.min(jnp.where(r == rmax, lane, S))
    idx = jnp.minimum(idx, S - 1)
    idx_s[0] = idx

    def ffn():
        idx = idx_s[0]
        base = pl.multiple_of((idx // 16) * 16, 16)
        tile = xn_v[pl.ds(base, 16), :].astype(f32)
        sub = jax.lax.broadcasted_iota(jnp.int32, tile.shape, 0)
        xs = jnp.sum(jnp.where(sub == idx - base, tile, 0.0), axis=0, keepdims=True)
        xs = jnp.broadcast_to(xs, (16, D)).astype(bf16)
        wg_copy.wait()
        gate = _dot(xs, wg_v[...], 1, 0)
        wu_copy.wait()
        up = _dot(xs, wu_v[...], 1, 0)
        hid = (gate * jax.nn.sigmoid(gate) * up).astype(bf16)
        wd_copy.wait()
        y = _dot(hid, wd_v[...], 1, 0)
        y_v[...] = y[0:8, :] * jax.nn.sigmoid(jnp.broadcast_to(rmax, (8, D)))

    nck = S // _CK
    steps = [(h, j) for h in range(HG * _GU) for j in range(nck)]

    NI = NG // _GU

    def qk_at(gi, q0, hh, j, qts):
        g, h = gi * _GU + hh // HG, hh % HG
        if hh not in qts:
            qts[hh] = qt_v[g, h * Dh:(h + 1) * Dh, pl.ds(q0, _BQ)]
        kh = k_v[g, j * _CK:(j + 1) * _CK, h * Dh:(h + 1) * Dh]
        p = jnp.exp2(_dot(kh, qts[hh], 1, 0))
        return p.reshape(_CK // 8, 8, _BQ).sum(axis=0), p.astype(bf16)

    def prefill(gi, q0, t, qts):
        pl_v[t], pp_v[t] = qk_at(gi, q0, *steps[t], qts)

    for t in range(_LAG):
        prefill(0, 0, t, {})

    def attn_fast(gi, q0, bad):
        qts, nqts = {}, {}
        last = gi == NI - 1
        ngi = jnp.where(last, 0, gi + 1)
        nq0 = pl.multiple_of(jnp.where(last, jnp.minimum(q0 + _BQ, S - _BQ), q0), _BQ)
        pend = {t: (pl_v[t], pp_v[t]) for t in range(_LAG)}
        o = l = None
        for t, (hh, j) in enumerate(steps):
            g, h = gi * _GU + hh // HG, hh % HG
            if t + _LAG < len(steps):
                pend[t + _LAG] = qk_at(gi, q0, *steps[t + _LAG], qts)
            else:
                prefill(ngi, nq0, t + _LAG - len(steps), nqts)
            ps, pb = pend.pop(t)
            pv = _dot(vt_v[g, h * Dh:(h + 1) * Dh, j * _CK:(j + 1) * _CK], pb, 1, 0)
            o = pv if j == 0 else o + pv
            l = ps if j == 0 else l + ps
            if j == nck - 1:
                l = l.sum(axis=0, keepdims=True)
                on = o / l
                ot_v[g, h * Dh:(h + 1) * Dh, :] = on.astype(bf16)
                ok = (l >= _L_LO) & (l <= _L_HI)
                ok = ok & (jnp.abs(on[0:8]) <= _BIG) & (jnp.abs(on[8:16]) <= _BIG)
                bad = jnp.where(ok, bad, 1.0)
        return bad

    def attn_safe(hh, q0):
        g = hh // HG
        r0 = pl.multiple_of((hh % HG) * Dh, Dh)
        qt = qt_v[g, :, pl.ds(q0, _BQ)]
        row = jax.lax.broadcasted_iota(jnp.int32, qt.shape, 0)
        qm = jnp.where((row >= r0) & (row < r0 + Dh), qt, jnp.zeros_like(qt))
        s = _dot(k_v[g], qm, 1, 0)
        p = jnp.exp2(s - jnp.max(s, axis=0, keepdims=True))
        l = jnp.sum(p, axis=0, keepdims=True)
        o = _dot(vt_v[g, pl.ds(r0, Dh), :], p.astype(bf16), 1, 0)
        ot_v[g, pl.ds(r0, Dh), :] = (o / l).astype(bf16)

    def out_copy(b, slot):
        return pltpu.make_async_copy(
            out_v.at[slot], out_hbm.at[0, pl.ds(b * _BQ, _BQ), :], osems.at[slot])

    def block(b, carry):
        q0 = pl.multiple_of(b * _BQ, _BQ)
        bad = jax.lax.fori_loop(0, NG // _GU, lambda g, bd: attn_fast(g, q0, bd),
                                jnp.zeros((8, _BQ), f32))

        @pl.when(jnp.max(bad) > 0.0)
        def _():
            jax.lax.fori_loop(0, _H, lambda hh, c: (attn_safe(hh, q0), c)[1], 0)

        @pl.when(b == 0)
        def _():
            wo_copy.wait()
            ffn()

        slot = b % 2

        @pl.when(b >= 2)
        def _():
            out_copy(b - 2, slot).wait()

        a = _dot(ot_v[...].reshape(D, _BQ), wo_v[...], 0, 0)
        rows = pl.ds(q0, _BQ)
        res = x_v[rows, :].astype(f32) + a + xn_v[rows, :].astype(f32)
        rid = jax.lax.broadcasted_iota(jnp.int32, (_BQ, D), 0) + q0
        res = res + jnp.where(rid == idx_s[0], y_v[0:1, :], 0.0)
        out_v[slot] = res.astype(bf16)
        out_copy(b, slot).start()
        return carry

    jax.lax.fori_loop(0, NB, block, 0)
    for b in range(max(NB - 2, 0), NB):
        out_copy(b, b % 2).wait()


@jax.jit
def pallas_parallel_sum__softmax_full_mha__moe_arch_mod__prompt_kernel(
    A_x: jax.Array,
    A_wqkv: jax.Array,
    A_wo: jax.Array,
    B_x: jax.Array,
    B_w_r: jax.Array,
    B_w_gate: jax.Array,
    B_w_up: jax.Array,
    B_w_down: jax.Array,
):
    del B_x
    _, S, D = A_x.shape
    F = B_w_gate.shape[1]
    NG = D // 128
    hbm = pl.BlockSpec(memory_space=pl.ANY)
    vmem = pl.BlockSpec(memory_space=pltpu.VMEM)
    scratch = [
        pltpu.VMEM((S, D), bf16),
        pltpu.VMEM((S, D), bf16),
        pltpu.VMEM((3, D, D), bf16),
        pltpu.VMEM((D, D), bf16),
        pltpu.VMEM((D, F), bf16),
        pltpu.VMEM((D, F), bf16),
        pltpu.VMEM((F, D), bf16),
        pltpu.VMEM((NG, S, 128), bf16),
        pltpu.VMEM((NG, 128, S), bf16),
        pltpu.VMEM((NG, 128, S), bf16),
        pltpu.VMEM((8, S), f32),
        pltpu.VMEM((NG, 128, _BQ), bf16),
        pltpu.VMEM((_LAG, _CK, _BQ), bf16),
        pltpu.VMEM((_LAG, 8, _BQ), f32),
        pltpu.VMEM((8, D), f32),
        pltpu.VMEM((2, _BQ, D), bf16),
        pltpu.SMEM((1,), jnp.int32),
        pltpu.SemaphoreType.DMA((S // _RC + 7,)),
        pltpu.SemaphoreType.DMA((2,)),
    ]
    return pl.pallas_call(
        _kernel,
        out_shape=jax.ShapeDtypeStruct(A_x.shape, A_x.dtype),
        in_specs=[hbm, hbm, hbm, vmem, hbm, hbm, hbm],
        out_specs=hbm,
        scratch_shapes=scratch,
        compiler_params=pltpu.CompilerParams(vmem_limit_bytes=100 * 2 ** 20),
    )(A_x, A_wqkv, A_wo, B_w_r, B_w_gate, B_w_up, B_w_down)
```
